```python
import jax
import jax.numpy as jnp

def _softmax(x, axis=-1):
    return jax.nn.softmax(x, axis=axis)
def _gelu(x):
    return jax.nn.gelu(x, approximate=True)
def _silu(x):
    return jax.nn.silu(x)
def _sigmoid(x):
    return jax.nn.sigmoid(x)
def _layernorm(x, axis=-1, eps=1e-5):
    m = jnp.mean(x, axis=axis, keepdims=True)
    v = jnp.var(x, axis=axis, keepdims=True)
    return (x - m) / jnp.sqrt(v + eps)
def _scatter_add(tgt, idx, src, axis=0):
    return tgt.at[idx].add(src)
def _segment_sum(src, seg, n):
    return jax.ops.segment_sum(src, seg, n)
class _Rng:
    def __init__(self, key):
        self._k = key
    def _next(self):
        self._k, sub = jax.random.split(self._k)
        return sub
    def normal(self, shape):
        return jax.random.normal(self._next(), shape, dtype=jnp.bfloat16)
    def randint(self, lo, hi, shape):
        return jax.random.randint(self._next(), shape, lo, hi, dtype=jnp.int32)
    def uniform(self, shape, lo=0.0, hi=1.0):
        return jax.random.uniform(self._next(), shape, jnp.bfloat16, lo, hi)
    def permutation(self, n):
        return jax.random.permutation(self._next(), n)


kernel_name = 'standalone__qk_norm__prompt'

def setup_inputs():
    _rng = _Rng(jax.random.key(int.from_bytes(__import__("os").urandom(4), "little")))
    _w = (lambda a: (lambda t: t.astype(jnp.bfloat16) if jnp.issubdtype(t.dtype, jnp.floating) else t)(jnp.asarray(a)))
    B, H, S, D = 2, 32, 2048, 1024
    Dh = D // H
    return {
        "q": _w((lambda *s: _rng.normal(s) * 0.05)(B, H, S, Dh)),
        "k": _w((lambda *s: _rng.normal(s) * 0.05)(B, H, S, Dh)),
        "v": _w((lambda *s: _rng.normal(s) * 0.05)(B, H, S, Dh)),
        "t": _w(jnp.abs((lambda *s: _rng.normal(s) * 0.05)(H)) + 1.0),
    }

def reference(q, k, v, t):
    eps = 1e-6
    qn = q / (jnp.sqrt((q * q).sum(axis=-1, keepdims=True)) + eps)
    kn = k / (jnp.sqrt((k * k).sum(axis=-1, keepdims=True)) + eps)
    logits = jnp.einsum('bhqd,bhkd->bhqk', qn, kn) * t[None, :, None, None]
    attn = _softmax(logits, axis=-1)
    return jnp.einsum('bhqk,bhkd->bhqd', attn, v)
```

```python
import jax
import jax.numpy as jnp
from jax.experimental import pallas as pl
from jax.experimental.pallas import tpu as pltpu

_LOG2E = 1.4426950408889634
_EPS = 1e-6
_T_SAFE = 16.0
_TILE = 128
_G = 4
_SKEW = 8
_END_SKEW = 24
_END_QT = 3
_NORM_SPAN = (10, 230)
_LINK_LAG = 12
_SLOW_BQ = 512
_SLOW_BK = 512

_f32 = jnp.float32
_bf16 = jnp.bfloat16
_u32 = jnp.uint32


def _make_kernel(n_heads, heads_per_batch, d, s):
    tile, grp = _TILE, _G
    nt = s // tile
    n_groups = n_heads // grp
    steps_per_head = nt * nt

    def normalize(x, scale):
        return x * (scale / (jnp.sqrt(jnp.sum(x * x, axis=0, keepdims=True)) + _EPS))

    def kernel(t_ref, q_hbm, k_hbm, v_hbm, o_hbm,
               q_v, k_v, v_v, o_v, kh_ref, qh_ref, ks_ref, qs_ref, sem_h, sem_r, sem_o):
        def head_copies(i):
            j = jnp.minimum(i, n_groups - 1)
            return [pltpu.make_async_copy(q_hbm.at[j * grp], q_v.at[i * grp], sem_h.at[i, 0]),
                    pltpu.make_async_copy(k_hbm.at[j * grp], k_v.at[i * grp], sem_h.at[i, 1])]

        def rest_copies(i):
            j = jnp.minimum(i, n_groups - 1)
            return [
                pltpu.make_async_copy(v_hbm.at[pl.ds(j * grp, grp)], v_v.at[pl.ds(i * grp, grp)],
                                      sem_r.at[i, 0]),
                pltpu.make_async_copy(q_hbm.at[pl.ds(j * grp + 1, grp - 1)],
                                      q_v.at[pl.ds(i * grp + 1, grp - 1)], sem_r.at[i, 1]),
                pltpu.make_async_copy(k_hbm.at[pl.ds(j * grp + 1, grp - 1)],
                                      k_v.at[pl.ds(i * grp + 1, grp - 1)], sem_r.at[i, 2]),
            ]

        def out_copy(i, g, n):
            return pltpu.make_async_copy(o_v.at[pl.ds(i * grp + g, n)],
                                         o_hbm.at[pl.ds(i * grp + g, n)], sem_o.at[i])

        def t_of(h):
            return t_ref[h % heads_per_batch].astype(_f32)

        def cols(i):
            return slice(i * tile, (i + 1) * tile)

        def store_handoff(h):
            scale = t_of(h) * _LOG2E
            for i in range(nt):
                qn = normalize(q_v[h, :, cols(i)].astype(_f32), scale).astype(_bf16)
                qh_ref[:, cols(i)] = pltpu.bitcast(qn, _u32)
                kn = normalize(k_v[h, :, cols(i)].astype(_f32), 1.0).T.astype(_bf16)
                kh_ref[i * (tile // 2):(i + 1) * (tile // 2), :] = pltpu.bitcast(kn, _u32)

        def fast_group(it):
            h0 = it * grp
            zero = jnp.full((8, 128), it >> 12, jnp.int32).astype(_u32)
            kn, qn, vt, state = {}, {}, {}, {}
            links, due, last_l = [], {}, [None]

            for i in range(nt):
                kn[0, i] = pltpu.bitcast(kh_ref[i * (tile // 2):(i + 1) * (tile // 2), :], _bf16)
                qn[0, i] = pltpu.bitcast(qh_ref[:, cols(i)], _bf16)

            def released(x):
                if last_l[0] is None:
                    return x
                z = jax.lax.bitcast_convert_type(last_l[0], _u32) & zero
                xb = pltpu.bitcast(x, _u32)
                xb = jnp.concatenate([xb[r:r + 8] | z for r in range(0, xb.shape[0], 8)], axis=0)
                return pltpu.bitcast(xb, _bf16)

            def and_bits(x):
                xb = pltpu.bitcast(x, _u32)
                m = xb[0:8, 0:d]
                for r in range(8, xb.shape[0], 8):
                    m = m & xb[r:r + 8, 0:d]
                return m

            def background(g):
                h = jnp.minimum(h0 + g, n_heads - 1)
                scale = []

                def q_piece(i):
                    if not scale:
                        scale.append(t_of(h) * _LOG2E)
                    x = normalize(released(q_v[h, :, cols(i)]).astype(_f32), scale[0]).astype(_bf16)
                    if g == grp:
                        qh_ref[:, cols(i)] = pltpu.bitcast(x, _u32)
                    else:
                        qn[g, i] = x
                    links.append(and_bits(x))

                def k_piece(i):
                    x = normalize(released(k_v[h, :, cols(i)]).astype(_f32), 1.0).T.astype(_bf16)
                    if g == grp:
                        kh_ref[i * (tile // 2):(i + 1) * (tile // 2), :] = pltpu.bitcast(x, _u32)
                    else:
                        kn[g, i] = x
                    links.append(and_bits(x))

                pieces = []
                for i in range(nt):
                    pieces += [(q_piece, i), (k_piece, i)]
                lo, hi = _NORM_SPAN
                return [(lo + (hi - lo) * n // len(pieces), f, i) for n, (f, i) in enumerate(pieces)]

            def qk(g, qt, kt, step):
                lhs = kn[g, kt]
                deps = due.pop(step, [])
                if deps:
                    m = deps[0]
                    for y in deps[1:]:
                        m = m & y
                    lb = pltpu.bitcast(lhs, _u32)
                    lb = jnp.concatenate([lb[0:8] | (m & zero[:, 0:d]), lb[8:]], axis=0)
                    lhs = pltpu.bitcast(lb, _bf16)
                return jnp.dot(lhs, qn[g, qt], preferred_element_type=_f32)

            def pv(g, qt, kt, s_tile):
                p = jnp.exp2(s_tile)
                l_new = jnp.sum(p.reshape(tile // 8, 8, tile), axis=0)
                if (g, kt) not in vt:
                    vt[g, kt] = v_v[h0 + g, :, cols(kt)]
                a_new = jnp.dot(vt[g, kt], p.astype(_bf16), preferred_element_type=_f32)
                last_l[0] = l_new
                if kt == 0:
                    state[g, qt] = (l_new, a_new)
                    return
                l, acc = state[g, qt]
                l, acc = l + l_new, acc + a_new
                state[g, qt] = (l, acc)
                if kt == nt - 1:
                    del state[g, qt]
                    l = jnp.sum(l, axis=0, keepdims=True)
                    o_v[h0 + g, :, cols(qt)] = (acc * (1.0 / l)).astype(o_v.dtype)
                    if qt == nt - 1:
                        out_copy(it, g, 1).start()

            pending = []
            for g in range(grp):
                events, n_done = background(g + 1), 0
                for qt in range(nt):
                    for kt in range(nt):
                        head_step = qt * nt + kt
                        step = g * steps_per_head + head_step
                        pending.append((g, qt, kt, qk(g, qt, kt, step)))
                        limit = _SKEW
                        if g == grp - 1 and qt >= nt - _END_QT:
                            pos = (qt - (nt - _END_QT)) * nt + kt
                            limit = _SKEW + (_END_SKEW - _SKEW) * pos // (_END_QT * nt)
                        while len(pending) > limit:
                            pv(*pending.pop(0))
                        while n_done < len(events) and events[n_done][0] <= head_step:
                            events[n_done][1](events[n_done][2])
                            n_done += 1
                        if links:
                            due.setdefault(step + _LINK_LAG, []).extend(links)
                            links.clear()
            for item in pending:
                pv(*item)

        def slow_group(it):
            h0 = it * grp
            bq, bk = _SLOW_BQ, _SLOW_BK

            def head(g, carry):
                h = h0 + g
                t = t_of(h)
                qs_ref[...] = normalize(q_v[h].astype(_f32), 1.0).astype(_bf16)
                ks_ref[...] = normalize(k_v[h].astype(_f32), 1.0).T.astype(_bf16)

                def q_block(qi, carry):
                    q0 = pl.multiple_of(qi * bq, bq)
                    qb = qs_ref[:, pl.ds(q0, bq)]

                    def k_block(ki, mla):
                        m, l, acc = mla
                        k0 = pl.multiple_of(ki * bk, bk)
                        x = jnp.dot(ks_ref[pl.ds(k0, bk), :], qb, preferred_element_type=_f32) * t
                        m_new = jnp.maximum(m, jnp.max(x, axis=0, keepdims=True))
                        alpha = jnp.exp(m - m_new)
                        p = jnp.exp(x - m_new)
                        l = alpha * l + jnp.sum(p, axis=0, keepdims=True)
                        acc = alpha * acc + jnp.dot(v_v[h, :, pl.ds(k0, bk)], p.astype(_bf16),
                                                    preferred_element_type=_f32)
                        return m_new, l, acc

                    init = (jnp.full((1, bq), -jnp.inf, _f32), jnp.zeros((1, bq), _f32),
                            jnp.zeros((d, bq), _f32))
                    _, l, acc = jax.lax.fori_loop(0, s // bk, k_block, init)
                    o_v[h, :, pl.ds(q0, bq)] = (acc / l).astype(o_v.dtype)
                    return carry

                jax.lax.fori_loop(0, s // bq, q_block, 0)
                return carry

            jax.lax.fori_loop(0, grp, head, 0)
            store_handoff(jnp.minimum(h0 + grp, n_heads - 1))
            out_copy(it, 0, grp).start()

        for c in head_copies(0) + rest_copies(0) + head_copies(1) + rest_copies(1):
            c.start()
        for c in head_copies(0):
            c.wait()
        store_handoff(0)

        def body(it, carry):
            for c in rest_copies(it) + head_copies(it + 1):
                c.wait()
            for c in head_copies(it + 2) + rest_copies(it + 2):
                c.start()
            t_max = jnp.abs(t_of(it * grp))
            for g in range(1, grp):
                t_max = jnp.maximum(t_max, jnp.abs(t_of(it * grp + g)))
            safe = t_max <= _T_SAFE
            pl.when(safe)(lambda: fast_group(it))
            pl.when(jnp.logical_not(safe))(lambda: slow_group(it))
            return carry

        jax.lax.fori_loop(0, n_groups, body, 0)

        for c in rest_copies(n_groups) + head_copies(n_groups + 1) + rest_copies(n_groups + 1):
            c.wait()
        for i in range(n_groups):
            out_copy(i, 0, grp).wait()

    return kernel


@jax.jit
def pallas_standalone__qk_norm__prompt_kernel(
    q: jax.Array,
    k: jax.Array,
    v: jax.Array,
    t: jax.Array,
):
    b, h, s, d = q.shape
    n_heads = b * h
    assert d == 32 and s % _SLOW_BQ == 0 and s % _SLOW_BK == 0 and n_heads % _G == 0
    assert (s // _TILE) ** 2 > _NORM_SPAN[1] + _LINK_LAG
    n_groups = n_heads // _G
    q_t, k_t, v_t = (jnp.swapaxes(x, 2, 3).reshape(n_heads, d, s) for x in (q, k, v))
    any_spec = pl.BlockSpec(memory_space=pl.ANY)
    in_buf = pltpu.VMEM((n_heads + 2 * _G, d, s), q.dtype)
    o_t = pl.pallas_call(
        _make_kernel(n_heads, h, d, s),
        in_specs=[pl.BlockSpec(memory_space=pltpu.SMEM), any_spec, any_spec, any_spec],
        out_specs=any_spec,
        out_shape=jax.ShapeDtypeStruct((n_heads, d, s), q.dtype),
        scratch_shapes=[
            in_buf, in_buf, in_buf,
            pltpu.VMEM((n_heads, d, s), q.dtype),
            pltpu.VMEM((s // 2, d), _u32),
            pltpu.VMEM((d // 2, s), _u32),
            pltpu.VMEM((s, d), _bf16),
            pltpu.VMEM((d, s), _bf16),
            pltpu.SemaphoreType.DMA((n_groups + 2, 2)),
            pltpu.SemaphoreType.DMA((n_groups + 2, 3)),
            pltpu.SemaphoreType.DMA((n_groups,)),
        ],
        compiler_params=pltpu.CompilerParams(vmem_limit_bytes=100 * 1024 * 1024),
    )(t, q_t, k_t, v_t)
    return jnp.swapaxes(o_t.reshape(b, h, d, s), 2, 3)
```

```python
import jax
import jax.numpy as jnp
from jax.experimental import pallas as pl
from jax.experimental.pallas import tpu as pltpu

_LOG2E = 1.4426950408889634
_EPS = 1e-6
_T_SAFE = 16.0
_TILE = 128
_G = 4
_SKEW = 8
_END_SKEW = 48
_END_QT = 5
_NORM_SPAN = (10, 230)
_LINK_LAG = 12
_SLOW_BQ = 512
_SLOW_BK = 512

_f32 = jnp.float32
_bf16 = jnp.bfloat16
_u32 = jnp.uint32


def _make_kernel(n_heads, heads_per_batch, d, s):
    tile, grp = _TILE, _G
    nt = s // tile
    n_groups = n_heads // grp
    steps_per_head = nt * nt

    def normalize(x, scale):
        return x * (scale / (jnp.sqrt(jnp.sum(x * x, axis=0, keepdims=True)) + _EPS))

    def kernel(t_hbm, q_hbm, k_hbm, v_hbm, o_hbm,
               q_v, k_v, v_v, o_v, kh_ref, qh_ref, ks_ref, qs_ref, t_ref,
               sem_h, sem_r, sem_o, sem_t):
        def head_copies(i):
            j = jnp.minimum(i, n_groups - 1)
            return [pltpu.make_async_copy(q_hbm.at[j * grp], q_v.at[i * grp], sem_h.at[i, 0]),
                    pltpu.make_async_copy(k_hbm.at[j * grp], k_v.at[i * grp], sem_h.at[i, 1])]

        def rest_copies(i):
            j = jnp.minimum(i, n_groups - 1)
            return [
                pltpu.make_async_copy(v_hbm.at[pl.ds(j * grp, grp)], v_v.at[pl.ds(i * grp, grp)],
                                      sem_r.at[i, 0]),
                pltpu.make_async_copy(q_hbm.at[pl.ds(j * grp + 1, grp - 1)],
                                      q_v.at[pl.ds(i * grp + 1, grp - 1)], sem_r.at[i, 1]),
                pltpu.make_async_copy(k_hbm.at[pl.ds(j * grp + 1, grp - 1)],
                                      k_v.at[pl.ds(i * grp + 1, grp - 1)], sem_r.at[i, 2]),
            ]

        def out_copy(i, g, n):
            return pltpu.make_async_copy(o_v.at[pl.ds(i * grp + g, n)],
                                         o_hbm.at[pl.ds(i * grp + g, n)], sem_o.at[i])

        def t_of(h):
            return t_ref[h % heads_per_batch].astype(_f32)

        def cols(i):
            return slice(i * tile, (i + 1) * tile)

        def store_handoff(h):
            scale = t_of(h) * _LOG2E
            for i in range(nt):
                qn = normalize(q_v[h, :, cols(i)].astype(_f32), scale).astype(_bf16)
                qh_ref[:, cols(i)] = pltpu.bitcast(qn, _u32)
                kn = normalize(k_v[h, :, cols(i)].astype(_f32), 1.0).T.astype(_bf16)
                kh_ref[i * (tile // 2):(i + 1) * (tile // 2), :] = pltpu.bitcast(kn, _u32)

        def fast_group(it):
            h0 = it * grp
            zero = jnp.full((8, 128), it >> 12, jnp.int32).astype(_u32)
            kn, qn, vt, state = {}, {}, {}, {}
            links, due, last_l = [], {}, [None]

            for i in range(nt):
                kn[0, i] = pltpu.bitcast(kh_ref[i * (tile // 2):(i + 1) * (tile // 2), :], _bf16)
                qn[0, i] = pltpu.bitcast(qh_ref[:, cols(i)], _bf16)

            def released(x):
                if last_l[0] is None:
                    return x
                z = jax.lax.bitcast_convert_type(last_l[0], _u32) & zero
                xb = pltpu.bitcast(x, _u32)
                xb = jnp.concatenate([xb[r:r + 8] | z for r in range(0, xb.shape[0], 8)], axis=0)
                return pltpu.bitcast(xb, _bf16)

            def and_bits(x):
                xb = pltpu.bitcast(x, _u32)
                m = xb[0:8, 0:d]
                for r in range(8, xb.shape[0], 8):
                    m = m & xb[r:r + 8, 0:d]
                return m

            def background(g):
                h = jnp.minimum(h0 + g, n_heads - 1)
                scale = []

                def q_piece(i):
                    if not scale:
                        scale.append(t_of(h) * _LOG2E)
                    x = normalize(released(q_v[h, :, cols(i)]).astype(_f32), scale[0]).astype(_bf16)
                    if g == grp:
                        qh_ref[:, cols(i)] = pltpu.bitcast(x, _u32)
                    else:
                        qn[g, i] = x
                    links.append(and_bits(x))

                def k_piece(i):
                    x = normalize(released(k_v[h, :, cols(i)]).astype(_f32), 1.0).T.astype(_bf16)
                    if g == grp:
                        kh_ref[i * (tile // 2):(i + 1) * (tile // 2), :] = pltpu.bitcast(x, _u32)
                    else:
                        kn[g, i] = x
                    links.append(and_bits(x))

                pieces = []
                for i in range(nt):
                    pieces += [(q_piece, i), (k_piece, i)]
                lo, hi = _NORM_SPAN
                return [(lo + (hi - lo) * n // len(pieces), f, i) for n, (f, i) in enumerate(pieces)]

            def qk(g, qt, kt, step):
                lhs = kn[g, kt]
                deps = due.pop(step, [])
                if deps:
                    m = deps[0]
                    for y in deps[1:]:
                        m = m & y
                    lb = pltpu.bitcast(lhs, _u32)
                    lb = jnp.concatenate([lb[0:8] | (m & zero[:, 0:d]), lb[8:]], axis=0)
                    lhs = pltpu.bitcast(lb, _bf16)
                return jnp.dot(lhs, qn[g, qt], preferred_element_type=_f32)

            def pv(g, qt, kt, s_tile):
                p = jnp.exp2(s_tile)
                l_new = jnp.sum(p.reshape(tile // 8, 8, tile), axis=0)
                if (g, kt) not in vt:
                    vt[g, kt] = v_v[h0 + g, :, cols(kt)]
                a_new = jnp.dot(vt[g, kt], p.astype(_bf16), preferred_element_type=_f32)
                last_l[0] = l_new
                if kt == 0:
                    state[g, qt] = (l_new, a_new)
                    return
                l, acc = state[g, qt]
                l, acc = l + l_new, acc + a_new
                state[g, qt] = (l, acc)
                if kt == nt - 1:
                    del state[g, qt]
                    l = jnp.sum(l, axis=0, keepdims=True)
                    o_v[h0 + g, :, cols(qt)] = (acc * (1.0 / l)).astype(o_v.dtype)
                    if qt == nt - 1 and g == grp - 2:
                        out_copy(it, 0, grp - 1).start()
                    if qt == nt - 1 and g == grp - 1:
                        out_copy(it, g, 1).start()

            pending = []
            for g in range(grp):
                events, n_done = background(g + 1), 0
                for qt in range(nt):
                    for kt in range(nt):
                        head_step = qt * nt + kt
                        step = g * steps_per_head + head_step
                        pending.append((g, qt, kt, qk(g, qt, kt, step)))
                        limit = _SKEW
                        if g == grp - 1 and qt >= nt - _END_QT:
                            pos = (qt - (nt - _END_QT)) * nt + kt
                            limit = _SKEW + (_END_SKEW - _SKEW) * pos // (_END_QT * nt)
                        while len(pending) > limit:
                            pv(*pending.pop(0))
                        while n_done < len(events) and events[n_done][0] <= head_step:
                            events[n_done][1](events[n_done][2])
                            n_done += 1
                        if links:
                            due.setdefault(step + _LINK_LAG, []).extend(links)
                            links.clear()
            for item in pending:
                pv(*item)

        def slow_group(it):
            h0 = it * grp
            bq, bk = _SLOW_BQ, _SLOW_BK

            def head(g, carry):
                h = h0 + g
                t = t_of(h)
                qs_ref[...] = normalize(q_v[h].astype(_f32), 1.0).astype(_bf16)
                ks_ref[...] = normalize(k_v[h].astype(_f32), 1.0).T.astype(_bf16)

                def q_block(qi, carry):
                    q0 = pl.multiple_of(qi * bq, bq)
                    qb = qs_ref[:, pl.ds(q0, bq)]

                    def k_block(ki, mla):
                        m, l, acc = mla
                        k0 = pl.multiple_of(ki * bk, bk)
                        x = jnp.dot(ks_ref[pl.ds(k0, bk), :], qb, preferred_element_type=_f32) * t
                        m_new = jnp.maximum(m, jnp.max(x, axis=0, keepdims=True))
                        alpha = jnp.exp(m - m_new)
                        p = jnp.exp(x - m_new)
                        l = alpha * l + jnp.sum(p, axis=0, keepdims=True)
                        acc = alpha * acc + jnp.dot(v_v[h, :, pl.ds(k0, bk)], p.astype(_bf16),
                                                    preferred_element_type=_f32)
                        return m_new, l, acc

                    init = (jnp.full((1, bq), -jnp.inf, _f32), jnp.zeros((1, bq), _f32),
                            jnp.zeros((d, bq), _f32))
                    _, l, acc = jax.lax.fori_loop(0, s // bk, k_block, init)
                    o_v[h, :, pl.ds(q0, bq)] = (acc / l).astype(o_v.dtype)
                    return carry

                jax.lax.fori_loop(0, s // bq, q_block, 0)
                return carry

            jax.lax.fori_loop(0, grp, head, 0)
            out_copy(it, 0, grp).start()

        t_copy = pltpu.make_async_copy(t_hbm, t_ref, sem_t)
        t_copy.start()
        for c in head_copies(0) + rest_copies(0) + head_copies(1):
            c.start()
        t_copy.wait()
        t_max = jnp.abs(t_of(0))
        for i in range(1, heads_per_batch):
            t_max = jnp.maximum(t_max, jnp.abs(t_of(i)))
        safe = t_max <= _T_SAFE
        for c in head_copies(0):
            c.wait()

        def loop(group_fn):
            def body(it, carry):
                for c in rest_copies(it) + head_copies(it + 1):
                    c.wait()
                for c in rest_copies(it + 1) + head_copies(it + 2):
                    c.start()
                group_fn(it)
                return carry

            jax.lax.fori_loop(0, n_groups, body, 0)

        @pl.when(safe)
        def _():
            store_handoff(0)
            loop(fast_group)

        @pl.when(jnp.logical_not(safe))
        def _():
            loop(slow_group)

        for c in rest_copies(n_groups) + head_copies(n_groups + 1):
            c.wait()
        for i in range(n_groups):
            out_copy(i, 0, grp).wait()

    return kernel


@jax.jit
def pallas_standalone__qk_norm__prompt_kernel(
    q: jax.Array,
    k: jax.Array,
    v: jax.Array,
    t: jax.Array,
):
    b, h, s, d = q.shape
    n_heads = b * h
    assert d == 32 and s % _SLOW_BQ == 0 and s % _SLOW_BK == 0 and n_heads % _G == 0
    assert (s // _TILE) ** 2 > _NORM_SPAN[1] + _LINK_LAG
    n_groups = n_heads // _G
    q_t, k_t, v_t = (jnp.swapaxes(x, 2, 3).reshape(n_heads, d, s) for x in (q, k, v))
    any_spec = pl.BlockSpec(memory_space=pl.ANY)
    in_buf = pltpu.VMEM((n_heads + 2 * _G, d, s), q.dtype)
    o_t = pl.pallas_call(
        _make_kernel(n_heads, h, d, s),
        in_specs=[any_spec, any_spec, any_spec, any_spec],
        out_specs=any_spec,
        out_shape=jax.ShapeDtypeStruct((n_heads, d, s), q.dtype),
        scratch_shapes=[
            in_buf, in_buf, in_buf,
            pltpu.VMEM((n_heads, d, s), q.dtype),
            pltpu.VMEM((s // 2, d), _u32),
            pltpu.VMEM((d // 2, s), _u32),
            pltpu.VMEM((s, d), _bf16),
            pltpu.VMEM((d, s), _bf16),
            pltpu.SMEM(t.shape, t.dtype),
            pltpu.SemaphoreType.DMA((n_groups + 2, 2)),
            pltpu.SemaphoreType.DMA((n_groups + 2, 3)),
            pltpu.SemaphoreType.DMA((n_groups,)),
            pltpu.SemaphoreType.DMA(()),
        ],
        compiler_params=pltpu.CompilerParams(vmem_limit_bytes=100 * 1024 * 1024,
                                             disable_bounds_checks=True),
    )(t, q_t, k_t, v_t)
    return jnp.swapaxes(o_t.reshape(b, h, d, s), 2, 3)
```

```python
import jax
import jax.numpy as jnp
from jax.experimental import pallas as pl
from jax.experimental.pallas import tpu as pltpu

_LOG2E = 1.4426950408889634
_EPS = 1e-6
_T_SAFE = 16.0
_TILE = 128
_G = 4
_SKEW = 8
_END_SKEW = 48
_END_QT = 5
_NORM_SPAN = (10, 230)
_LINK_LAG = 12
_SLOW_BQ = 512
_SLOW_BK = 512

_f32 = jnp.float32
_bf16 = jnp.bfloat16
_u32 = jnp.uint32


def _make_kernel(n_heads, heads_per_batch, d, s):
    tile, grp = _TILE, _G
    nt = s // tile
    n_groups = n_heads // grp
    steps_per_head = nt * nt

    def normalize(x, scale):
        return x * (scale / (jnp.sqrt(jnp.sum(x * x, axis=0, keepdims=True)) + _EPS))

    def kernel(t_hbm, q_hbm, k_hbm, v_hbm, o_hbm,
               q_v, k_v, v_v, o_v, kh_ref, qh_ref, ks_ref, qs_ref, t_ref,
               sem_first, sem_in, sem_out):
        def head_copies(i, sem=sem_in):
            j = jnp.minimum(i, n_groups - 1)
            return [pltpu.make_async_copy(q_hbm.at[j * grp], q_v.at[i * grp], sem),
                    pltpu.make_async_copy(k_hbm.at[j * grp], k_v.at[i * grp], sem)]

        def rest_copies(i):
            j = jnp.minimum(i, n_groups - 1)
            return [
                pltpu.make_async_copy(v_hbm.at[pl.ds(j * grp, grp)], v_v.at[pl.ds(i * grp, grp)],
                                      sem_in),
                pltpu.make_async_copy(q_hbm.at[pl.ds(j * grp + 1, grp - 1)],
                                      q_v.at[pl.ds(i * grp + 1, grp - 1)], sem_in),
                pltpu.make_async_copy(k_hbm.at[pl.ds(j * grp + 1, grp - 1)],
                                      k_v.at[pl.ds(i * grp + 1, grp - 1)], sem_in),
            ]

        def out_copy(i, g, n):
            return pltpu.make_async_copy(o_v.at[pl.ds(i * grp + g, n)],
                                         o_hbm.at[pl.ds(i * grp + g, n)], sem_out)

        def t_of(h):
            return t_ref[h % heads_per_batch].astype(_f32)

        def cols(i):
            return slice(i * tile, (i + 1) * tile)

        def store_handoff(h):
            scale = t_of(h) * _LOG2E
            for i in range(nt):
                qn = normalize(q_v[h, :, cols(i)].astype(_f32), scale).astype(_bf16)
                qh_ref[:, cols(i)] = pltpu.bitcast(qn, _u32)
                kn = normalize(k_v[h, :, cols(i)].astype(_f32), 1.0).T.astype(_bf16)
                kh_ref[i * (tile // 2):(i + 1) * (tile // 2), :] = pltpu.bitcast(kn, _u32)

        def fast_group(it):
            h0 = it * grp
            zero = jnp.full((8, 128), it >> 12, jnp.int32).astype(_u32)
            kn, qn, vt, state = {}, {}, {}, {}
            links, due, last_l = [], {}, [None]

            for i in range(nt):
                kn[0, i] = pltpu.bitcast(kh_ref[i * (tile // 2):(i + 1) * (tile // 2), :], _bf16)
                qn[0, i] = pltpu.bitcast(qh_ref[:, cols(i)], _bf16)

            def released(x):
                if last_l[0] is None:
                    return x
                z = jax.lax.bitcast_convert_type(last_l[0], _u32) & zero
                xb = pltpu.bitcast(x, _u32)
                xb = jnp.concatenate([xb[r:r + 8] | z for r in range(0, xb.shape[0], 8)], axis=0)
                return pltpu.bitcast(xb, _bf16)

            def and_bits(x):
                xb = pltpu.bitcast(x, _u32)
                m = xb[0:8, 0:d]
                for r in range(8, xb.shape[0], 8):
                    m = m & xb[r:r + 8, 0:d]
                return m

            def background(g):
                h = jnp.minimum(h0 + g, n_heads - 1)
                scale = []

                def q_piece(i):
                    if not scale:
                        scale.append(t_of(h) * _LOG2E)
                    x = normalize(released(q_v[h, :, cols(i)]).astype(_f32), scale[0]).astype(_bf16)
                    if g == grp:
                        qh_ref[:, cols(i)] = pltpu.bitcast(x, _u32)
                    else:
                        qn[g, i] = x
                    links.append(and_bits(x))

                def k_piece(i):
                    x = normalize(released(k_v[h, :, cols(i)]).astype(_f32), 1.0).T.astype(_bf16)
                    if g == grp:
                        kh_ref[i * (tile // 2):(i + 1) * (tile // 2), :] = pltpu.bitcast(x, _u32)
                    else:
                        kn[g, i] = x
                    links.append(and_bits(x))

                pieces = []
                for i in range(nt):
                    pieces += [(q_piece, i), (k_piece, i)]
                lo, hi = _NORM_SPAN
                return [(lo + (hi - lo) * n // len(pieces), f, i) for n, (f, i) in enumerate(pieces)]

            def qk(g, qt, kt, step):
                lhs = kn[g, kt]
                deps = due.pop(step, [])
                if deps:
                    m = deps[0]
                    for y in deps[1:]:
                        m = m & y
                    lb = pltpu.bitcast(lhs, _u32)
                    lb = jnp.concatenate([lb[0:8] | (m & zero[:, 0:d]), lb[8:]], axis=0)
                    lhs = pltpu.bitcast(lb, _bf16)
                return jnp.dot(lhs, qn[g, qt], preferred_element_type=_f32)

            def pv(g, qt, kt, s_tile):
                p = jnp.exp2(s_tile)
                l_new = jnp.sum(p.reshape(tile // 8, 8, tile), axis=0)
                if (g, kt) not in vt:
                    vt[g, kt] = v_v[h0 + g, :, cols(kt)]
                a_new = jnp.dot(vt[g, kt], p.astype(_bf16), preferred_element_type=_f32)
                last_l[0] = l_new
                if kt == 0:
                    state[g, qt] = (l_new, a_new)
                    return
                l, acc = state[g, qt]
                l, acc = l + l_new, acc + a_new
                state[g, qt] = (l, acc)
                if kt == nt - 1:
                    del state[g, qt]
                    l = jnp.sum(l, axis=0, keepdims=True)
                    o_v[h0 + g, :, cols(qt)] = (acc * (1.0 / l)).astype(o_v.dtype)
                    if qt == nt - 1 and g == grp - 2:
                        out_copy(it, 0, grp - 1).start()
                    if qt == nt - 1 and g == grp - 1:
                        out_copy(it, g, 1).start()

            pending = []
            for g in range(grp):
                events, n_done = background(g + 1), 0
                for qt in range(nt):
                    for kt in range(nt):
                        head_step = qt * nt + kt
                        step = g * steps_per_head + head_step
                        pending.append((g, qt, kt, qk(g, qt, kt, step)))
                        limit = _SKEW
                        if g == grp - 1 and qt >= nt - _END_QT:
                            pos = (qt - (nt - _END_QT)) * nt + kt
                            limit = _SKEW + (_END_SKEW - _SKEW) * pos // (_END_QT * nt)
                        while len(pending) > limit:
                            pv(*pending.pop(0))
                        while n_done < len(events) and events[n_done][0] <= head_step:
                            events[n_done][1](events[n_done][2])
                            n_done += 1
                        if links:
                            due.setdefault(step + _LINK_LAG, []).extend(links)
                            links.clear()
            for item in pending:
                pv(*item)

        def slow_group(it):
            h0 = it * grp
            bq, bk = _SLOW_BQ, _SLOW_BK

            def head(g, carry):
                h = h0 + g
                t = t_of(h)
                qs_ref[...] = normalize(q_v[h].astype(_f32), 1.0).astype(_bf16)
                ks_ref[...] = normalize(k_v[h].astype(_f32), 1.0).T.astype(_bf16)

                def q_block(qi, carry):
                    q0 = pl.multiple_of(qi * bq, bq)
                    qb = qs_ref[:, pl.ds(q0, bq)]

                    def k_block(ki, mla):
                        m, l, acc = mla
                        k0 = pl.multiple_of(ki * bk, bk)
                        x = jnp.dot(ks_ref[pl.ds(k0, bk), :], qb, preferred_element_type=_f32) * t
                        m_new = jnp.maximum(m, jnp.max(x, axis=0, keepdims=True))
                        alpha = jnp.exp(m - m_new)
                        p = jnp.exp(x - m_new)
                        l = alpha * l + jnp.sum(p, axis=0, keepdims=True)
                        acc = alpha * acc + jnp.dot(v_v[h, :, pl.ds(k0, bk)], p.astype(_bf16),
                                                    preferred_element_type=_f32)
                        return m_new, l, acc

                    init = (jnp.full((1, bq), -jnp.inf, _f32), jnp.zeros((1, bq), _f32),
                            jnp.zeros((d, bq), _f32))
                    _, l, acc = jax.lax.fori_loop(0, s // bk, k_block, init)
                    o_v[h, :, pl.ds(q0, bq)] = (acc / l).astype(o_v.dtype)
                    return carry

                jax.lax.fori_loop(0, s // bq, q_block, 0)
                return carry

            jax.lax.fori_loop(0, grp, head, 0)
            out_copy(it, 0, grp).start()

        first = [pltpu.make_async_copy(t_hbm, t_ref, sem_first)] + head_copies(0, sem_first)
        for c in first + rest_copies(0) + head_copies(1):
            c.start()
        for c in first:
            c.wait()
        t_max = jnp.abs(t_of(0))
        for i in range(1, heads_per_batch):
            t_max = jnp.maximum(t_max, jnp.abs(t_of(i)))
        safe = t_max <= _T_SAFE

        def loop(group_fn):
            def body(it, carry):
                for c in rest_copies(it) + head_copies(it + 1):
                    c.wait()
                for c in rest_copies(it + 1) + head_copies(it + 2):
                    c.start()
                group_fn(it)
                return carry

            jax.lax.fori_loop(0, n_groups, body, 0)

        @pl.when(safe)
        def _():
            store_handoff(0)
            loop(fast_group)

        @pl.when(jnp.logical_not(safe))
        def _():
            loop(slow_group)

        for c in rest_copies(n_groups) + head_copies(n_groups + 1):
            c.wait()
        pltpu.make_async_copy(o_v, o_hbm, sem_out).wait()

    return kernel


@jax.jit
def pallas_standalone__qk_norm__prompt_kernel(
    q: jax.Array,
    k: jax.Array,
    v: jax.Array,
    t: jax.Array,
):
    b, h, s, d = q.shape
    n_heads = b * h
    assert d == 32 and s % _SLOW_BQ == 0 and s % _SLOW_BK == 0 and n_heads % _G == 0
    assert (s // _TILE) ** 2 > _NORM_SPAN[1] + _LINK_LAG
    q_t, k_t, v_t = (jnp.swapaxes(x, 2, 3).reshape(n_heads, d, s) for x in (q, k, v))
    any_spec = pl.BlockSpec(memory_space=pl.ANY)
    in_buf = pltpu.VMEM((n_heads + 2 * _G, d, s), q.dtype)
    o_t = pl.pallas_call(
        _make_kernel(n_heads, h, d, s),
        in_specs=[any_spec, any_spec, any_spec, any_spec],
        out_specs=any_spec,
        out_shape=jax.ShapeDtypeStruct((n_heads, d, s), q.dtype),
        scratch_shapes=[
            in_buf, in_buf, in_buf,
            pltpu.VMEM((n_heads, d, s), q.dtype),
            pltpu.VMEM((s // 2, d), _u32),
            pltpu.VMEM((d // 2, s), _u32),
            pltpu.VMEM((s, d), _bf16),
            pltpu.VMEM((d, s), _bf16),
            pltpu.SMEM(t.shape, t.dtype),
            pltpu.SemaphoreType.DMA(()),
            pltpu.SemaphoreType.DMA(()),
            pltpu.SemaphoreType.DMA(()),
        ],
        compiler_params=pltpu.CompilerParams(vmem_limit_bytes=100 * 1024 * 1024,
                                             disable_bounds_checks=True),
    )(t, q_t, k_t, v_t)
    return jnp.swapaxes(o_t.reshape(b, h, d, s), 2, 3)
```
